```python
import os as _os
_os.environ.setdefault("JAX_PLATFORMS", "cpu")
import jax
import jax.numpy as jnp

def _softmax(x, axis=-1):
    return jax.nn.softmax(x, axis=axis)
def _gelu(x):
    return jax.nn.gelu(x, approximate=True)
def _silu(x):
    return jax.nn.silu(x)
def _sigmoid(x):
    return jax.nn.sigmoid(x)
def _layernorm(x, axis=-1, eps=1e-5):
    m = jnp.mean(x, axis=axis, keepdims=True)
    v = jnp.var(x, axis=axis, keepdims=True)
    return (x - m) / jnp.sqrt(v + eps)
def _scatter_add(tgt, idx, src, axis=0):
    return tgt.at[idx].add(src)
def _segment_sum(src, seg, n):
    return jax.ops.segment_sum(src, seg, n)
class _Rng:
    def __init__(self, key):
        self._k = key
    def _next(self):
        self._k, sub = jax.random.split(self._k)
        return sub
    def normal(self, shape):
        return jax.random.normal(self._next(), shape, dtype=jnp.bfloat16)
    def randint(self, lo, hi, shape):
        return jax.random.randint(self._next(), shape, lo, hi, dtype=jnp.int32)
    def uniform(self, shape, lo=0.0, hi=1.0):
        return jax.random.uniform(self._next(), shape, jnp.bfloat16, lo, hi)
    def permutation(self, n):
        return jax.random.permutation(self._next(), n)


kernel_name = 'concat_heads__mha_block_cached__gqa_block_cached__decode'

def setup_inputs():
    _rng = _Rng(jax.random.key(int.from_bytes(__import__("os").urandom(4), "little")))
    _w = (lambda a: (lambda t: t.astype(jnp.bfloat16) if jnp.issubdtype(t.dtype, jnp.floating) else t)(jnp.asarray(a)))
    def _A_setup():
        B, Sq, D = 1, 1, 512
        H, Sk, Dh = 32, 4096, 128
        return {
            "x": _w((lambda *s: _rng.normal(s) * 0.8)(B, Sq, D)),
            "k_cache": _w((lambda *s: _rng.normal(s) * 0.8)(B, H, Sk, Dh)),
            "v_cache": _w((lambda *s: _rng.normal(s) * 0.05)(B, H, Sk, Dh)),
            "wq": _w((lambda *s: _rng.normal(s) * 0.8)(D, H * Dh) * (D ** -0.5)),
            "wo": _w((lambda *s: _rng.normal(s) * 0.05)(H * Dh, D) * ((H * Dh) ** -0.5)),
        }
    _A_in = _A_setup()

    def _B_setup():
        B, Sq, D = 1, 1, 512
        Hq, Hkv, Sk, Dh = 32, 32, 4096, 128
        assert Hq % Hkv == 0, (Hq, Hkv)
        return {
            "x": _w((lambda *s: _rng.normal(s) * 0.8)(B, Sq, D)),
            "k_cache": _w((lambda *s: _rng.normal(s) * 0.8)(B, Hkv, Sk, Dh)),
            "v_cache": _w((lambda *s: _rng.normal(s) * 0.05)(B, Hkv, Sk, Dh)),
            "wq": _w((lambda *s: _rng.normal(s) * 0.8)(D, Hq * Dh) * (D ** -0.5)),
            "wo": _w((lambda *s: _rng.normal(s) * 0.05)(Hq * Dh, D) * ((Hq * Dh) ** -0.5)),
        }
    _B_in = _B_setup()

    return {
        "A_x": _A_in["x"],
        "A_k_cache": _A_in["k_cache"],
        "A_v_cache": _A_in["v_cache"],
        "A_wq": _A_in["wq"],
        "A_wo": _A_in["wo"],
        "B_x": _B_in["x"],
        "B_k_cache": _B_in["k_cache"],
        "B_v_cache": _B_in["v_cache"],
        "B_wq": _B_in["wq"],
        "B_wo": _B_in["wo"],
    }

def reference(A_x, A_k_cache, A_v_cache, A_wq, A_wo, B_x, B_k_cache, B_v_cache, B_wq, B_wo):
    def _A_ref(x, k_cache, v_cache, wq, wo):
        B, Sq, D = x.shape
        H, Dh = 32, 128
        q = (lambda x, *d: x.transpose(*d))((x @ wq).reshape(B, Sq, H, Dh), 0, 2, 1, 3)
        scores = jnp.einsum("bhqd,bhkd->bhqk", q, k_cache) * (Dh ** -0.5)
        p = _softmax(scores, axis=-1)
        o = jnp.einsum("bhqk,bhkd->bhqd", p, v_cache)
        return (lambda x, *d: x.transpose(*d))(o, 0, 2, 1, 3).reshape(B, Sq, H * Dh) @ wo

    def _B_ref(x, k_cache, v_cache, wq, wo):
        B, Sq, D = x.shape
        Hq, Dh = 32, 128
        Hkv = k_cache.shape[1]
        rep = Hq // Hkv
        q = (lambda x, *d: x.transpose(*d))((x @ wq).reshape(B, Sq, Hq, Dh), 0, 2, 1, 3)
        k = jnp.repeat(k_cache, rep, axis=1)
        v = jnp.repeat(v_cache, rep, axis=1)
        scores = jnp.einsum("bhqd,bhkd->bhqk", q, k) * (Dh ** -0.5)
        p = _softmax(scores, axis=-1)
        o = jnp.einsum("bhqk,bhkd->bhqd", p, v)
        return (lambda x, *d: x.transpose(*d))(o, 0, 2, 1, 3).reshape(B, Sq, Hq * Dh) @ wo

    a = _A_ref(A_x, A_k_cache, A_v_cache, A_wq, A_wo)
    b = _B_ref(B_x, B_k_cache, B_v_cache, B_wq, B_wo)
    return jnp.concatenate([a, b], axis=-1)
```

```python
import functools

import jax
import jax.numpy as jnp
from jax import lax
import jax.experimental.pallas as pl
import jax.experimental.pallas.tpu as pltpu

D = 512
H = 32
SK = 4096
DH = 128
G = 8
NG = H // G
T = 128
NT = SK // T
NT_DIMS = (((1,), (1,)), ((), ()))


def make(lag=16, nslot=32, interleave=True, nochk=True, unroll=1):
    assert NT % lag == 0 and nslot > lag and NT % nslot == 0 or nslot % NT == 0
    f32, bf16 = jnp.float32, jnp.bfloat16

    def kernel(ax, ak, av, awq, awo, bx, bk, bv, bwq, bwo, out_ref,
               ring, wq_buf, wo_buf, x_buf, q_buf, s_buf, o_buf, sems, xsem):
        xs, ks, vs, wqs, wos = (ax, bx), (ak, bk), (av, bv), (awq, bwq), (awo, bwo)
        row = lax.broadcasted_iota(jnp.int32, (G, DH), 0)

        def issue_wq(t):
            c, r = t // 8, t % 8
            def piece(j):
                b, s = j % 2, j // 2
                idx = (pl.ds(pl.multiple_of(128 * s + 16 * r, 16), 16), pl.ds(pl.multiple_of(1024 * c, 1024), 1024))
                pltpu.make_async_copy(wqs[b].at[idx], wq_buf.at[b].at[idx], sems.at[t % nslot]).start(priority=j % 2)
            return piece

        def issue_kv(src, g, t):
            def piece(j):
                pltpu.make_async_copy(
                    src.at[0, g * G + j, pl.ds(pl.multiple_of(t * T, T), T)],
                    ring.at[t % nslot, j], sems.at[t % nslot]).start(priority=j % 2)
            return piece

        def issue_wo(t):
            def piece(j):
                b, s = j % 2, j // 2
                idx = pl.ds(pl.multiple_of(1024 * s + 32 * t, 32), 32)
                pltpu.make_async_copy(wos[b].at[idx], wo_buf.at[b, idx], sems.at[t % nslot]).start(priority=j % 2)
            return piece

        def wait(t):
            slot = t % nslot
            pltpu.make_async_copy(ring.at[slot], ring.at[slot], sems.at[slot]).wait()

        def run(issue, work):
            outs = []
            if not interleave and issue is not None:
                for j in range(G):
                    issue(j)
            for j in range(G):
                if interleave and issue is not None:
                    issue(j)
                if work is not None:
                    outs.append(work(j))
            return outs

        def diag(outs):
            r = outs[0]
            for j in range(1, G):
                r = jnp.where(row == j, outs[j], r)
            return r

        def loop(lo, hi, body, init=None):
            return lax.fori_loop(lo, hi, body, init, unroll=unroll)

        def pro(t, _):
            run(issue_wq(t), None)
        pro(0, None)
        xc = [pltpu.make_async_copy(xs[b].at[0], x_buf.at[b], xsem) for b in range(2)]
        for c in xc:
            c.start()
        lax.fori_loop(1, lag, pro, None)
        for c in xc:
            c.wait()

        def wq_stream(t, _):
            wait(t)
            run(issue_wq(t + lag), None)
        if lag < NT:
            lax.fori_loop(0, NT - lag, wq_stream, None)

        per = 16 // lag if lag <= 16 else 1

        def q_round(t, _):
            wait(t)
            u = t - (NT - lag)
            run(issue_kv(ks[0], 0, u), None)
        lax.fori_loop(NT - lag, NT, q_round, None)

        def q_unit(u, _):
            b, c = u // NG, u % NG
            x8 = jnp.broadcast_to(x_buf[b].astype(f32), (G, D)).astype(bf16)
            outs = [jnp.dot(x8, wq_buf[b, :, pl.ds(pl.multiple_of(1024 * c + DH * j, DH), DH)], preferred_element_type=f32)
                    for j in range(G)]
            q_buf[u] = diag(outs)
        lax.fori_loop(0, 2 * NG, q_unit, None)

        def k_round(q, issue, t, m):
            wait(t)
            slot = t % nslot
            outs = run(issue, lambda j: lax.dot_general(q, ring[slot, j], NT_DIMS, preferred_element_type=f32))
            s = diag(outs) * (DH ** -0.5)
            s_buf[t] = s
            return jnp.maximum(m, s)

        def v_round(m, issue, t, carry):
            l, acc = carry
            wait(t)
            slot = t % nslot
            p = jnp.exp(s_buf[t] - m)
            pb = p.astype(bf16)
            outs = run(issue, lambda j: jnp.dot(pb, ring[slot, j], preferred_element_type=f32))
            return l + p, acc + diag(outs)

        def group(b, g, last):
            q = q_buf[b * NG + g].astype(bf16)
            m = jnp.full((G, T), -jnp.inf, f32)
            if lag < NT:
                m = loop(0, NT - lag, lambda t, m: k_round(q, issue_kv(ks[b], g, t + lag), t, m), m)
            m = loop(NT - lag, NT, lambda t, m: k_round(q, issue_kv(vs[b], g, t + lag - NT), t, m), m)
            m = jnp.broadcast_to(jnp.max(m, axis=1, keepdims=True), (G, T))
            c = (jnp.zeros((G, T), f32), jnp.zeros((G, DH), f32))
            if lag < NT:
                c = loop(0, NT - lag, lambda t, c: v_round(m, issue_kv(vs[b], g, t + lag), t, c), c)
            if not last:
                nxt = lambda u: issue_kv(ks[b], g + 1, u)
            elif b == 0:
                nxt = lambda u: issue_kv(ks[1], 0, u)
            else:
                nxt = issue_wo
            l, acc = loop(NT - lag, NT, lambda t, c: v_round(m, nxt(t + lag - NT), t, c), c)
            o_buf[b * NG + g] = acc / jnp.sum(l, axis=1, keepdims=True)

        for b in range(2):
            lax.fori_loop(0, NG - 1, lambda g, _: group(b, g, False), None)
            group(b, NG - 1, True)

        def wo_unit(issue, hh, accs):
            for r in range(4):
                wait(4 * hh + r)
            accs = list(accs)
            for r in range(4):
                if issue is not None:
                    run(issue(4 * hh + r), None)
                for b in range(2):
                    o = o_buf[b * NG + r, pl.ds(hh, 1), :].astype(bf16)
                    w = wo_buf[b, pl.ds(pl.multiple_of(1024 * r + DH * hh, DH), DH), :]
                    accs[b] = accs[b] + jnp.dot(o, w, preferred_element_type=f32)
            return tuple(accs)

        accs = (jnp.zeros((1, D), f32),) * 2
        n1 = (NT - lag) // 4
        if n1:
            accs = lax.fori_loop(0, n1, functools.partial(wo_unit, lambda t: issue_wo(t + lag)), accs)
        accs = lax.fori_loop(n1, G, functools.partial(wo_unit, None), accs)
        out_ref[0] = jnp.concatenate(accs, axis=1).astype(out_ref.dtype)

    def f(A_x, A_k_cache, A_v_cache, A_wq, A_wo, B_x, B_k_cache, B_v_cache, B_wq, B_wo):
        return pl.pallas_call(
            kernel,
            out_shape=jax.ShapeDtypeStruct((1, 1, 2 * D), A_x.dtype),
            in_specs=[pl.BlockSpec(memory_space=pltpu.HBM)] * 10,
            out_specs=pl.BlockSpec(memory_space=pltpu.VMEM),
            scratch_shapes=[
                pltpu.VMEM((nslot, G, T, DH), bf16),
                pltpu.VMEM((2, D, H * DH), bf16),
                pltpu.VMEM((2, H * DH, D), bf16),
                pltpu.VMEM((2, 1, D), bf16),
                pltpu.VMEM((2 * NG, G, DH), f32),
                pltpu.VMEM((NT, G, T), f32),
                pltpu.VMEM((2 * NG, G, DH), f32),
                pltpu.SemaphoreType.DMA((nslot,)),
                pltpu.SemaphoreType.DMA(()),
            ],
            compiler_params=pltpu.CompilerParams(
                vmem_limit_bytes=48 * 1024 * 1024,
                disable_bounds_checks=nochk, disable_semaphore_checks=nochk),
        )(A_x, A_k_cache, A_v_cache, A_wq, A_wo, B_x, B_k_cache, B_v_cache, B_wq, B_wo)
    return f


@jax.jit
def pallas_concat_heads__mha_block_cached__gqa_block_cached__decode_kernel(
    A_x, A_k_cache, A_v_cache, A_wq, A_wo, B_x, B_k_cache, B_v_cache, B_wq, B_wo):
    return make()(A_x, A_k_cache, A_v_cache, A_wq, A_wo, B_x, B_k_cache, B_v_cache, B_wq, B_wo)
```

```python
import functools

import jax
import jax.numpy as jnp
from jax import lax
import jax.experimental.pallas as pl
import jax.experimental.pallas.tpu as pltpu

D = 512
H = 32
SK = 4096
DH = 128
G = 16
P = G // 2
T = 64
NT = SK // T
NGRP = 2 * H // G
NC = D // DH
LAG = 12
NSLOT = 16
SKEW = 7
KV_ORDER = (0, 4, 1, 5, 2, 6, 3, 7)
W_ORDER = (0, 4, 1, 5, 2, 6, 3)


def _kernel(ax, ak, av, awq, awo, bx, bk, bv, bwq, bwo, out_ref,
            ring, wq_buf, wo_buf, x_buf, xg_buf, s_buf, y_buf, o_buf, sems, x_sem):
    f32, bf16 = jnp.float32, jnp.bfloat16
    row = lax.broadcasted_iota(jnp.int32, (G, DH), 0)
    pair_of_row = row & (P - 1)
    even_lanes = lax.broadcasted_iota(jnp.int32, (P, 2 * T), 1) < T
    zeros = jnp.zeros((G, DH), f32)

    def copy(src, dst, t):
        return pltpu.make_async_copy(src, dst, sems.at[t & (NSLOT - 1)])

    def wo_copy(b, half, i, t):
        return copy((awo, bwo)[b].at[half, :, i], wo_buf.at[2 * b + half, i], t)

    def weight_copies(t):
        grp = t >> 5
        rows = pl.ds(pl.multiple_of(((t >> 1) & 15) * 8, 8), 8)
        cols = pl.ds(pl.multiple_of((t & 1) * 1024, 1024), 1024)
        src_cols = pl.ds(pl.multiple_of((2 * grp + (t & 1)) * 1024, 1024), 1024)
        copies = []
        for n in W_ORDER:
            b, is_wo, half = n // 4, (n // 2) % 2, n % 2
            if is_wo:
                copies.append(wo_copy(b, half, t, t))
            else:
                copies.append(copy((awq, bwq)[b].at[half, :, rows, src_cols],
                                   wq_buf.at[2 * b + grp, half, :, rows, cols], t))
        return copies

    def start_weights(t):
        for j, c in enumerate(weight_copies(t)):
            c.start(priority=1 - j % 2)

    def start_kv(src, grp, t, j):
        n = KV_ORDER[j]
        keys = (t - SKEW * (j % 2)) & (NT - 1)
        copy(src.at[P * grp + n, :, keys], ring.at[t & (NSLOT - 1), n], t).start(priority=1 - j % 2)

    def start_ahead(phase, t, j, may_end):
        phase, t = phase + ((t + LAG) >> 6), (t + LAG) & (NT - 1)
        source = (phase & 1) | ((phase >> 2) << 1)
        for n, src in enumerate((ak, av, bk, bv)):
            pl.when(source == n)(functools.partial(start_kv, src, (phase >> 1) & 1, t, j))
        if may_end:
            @pl.when((source == 4) & (t < P))
            def _():
                wo_copy(1, 1, 8 * t + j, t).start(priority=int(j % 4 != 3))

    def wait_kv(t):
        slot = ring.at[t & (NSLOT - 1)]
        copy(slot, slot, t).wait()

    def tile(t, n):
        return ring[t & (NSLOT - 1), n].reshape(2 * T, DH)

    def own_rows(outs):
        r = outs[0]
        for n in range(1, P):
            r = jnp.where(pair_of_row == n, outs[n], r)
        return r

    def row_of(h):
        return (h >> 1) + P * (h & 1)

    def q_tile(grp, t):
        h, c = t >> 2, t & 3
        w = wq_buf[grp, c >> 1, c & 1, :, pl.ds(pl.multiple_of(h * DH, DH), DH)]
        q = jnp.dot(xg_buf[grp >> 1, c], w, preferred_element_type=f32)
        return jnp.where(row == row_of(h), q, 0.0)

    start_weights(0)
    x_copies = [pltpu.make_async_copy(x.at[0], x_buf.at[b], x_sem) for b, x in enumerate((ax, bx))]
    for c in x_copies:
        c.start()

    def weight_step(i, q):
        @pl.when(i >= LAG)
        def _():
            for c in weight_copies(i - LAG):
                c.wait()

        pl.when(i < NT)(functools.partial(start_weights, i))

        @pl.when(i >= NT)
        def _():
            for j in range(P):
                start_kv(ak, 0, i - NT, j)

        @pl.when(i == LAG)
        def _():
            for c in x_copies:
                c.wait()
            for b in range(2):
                x = x_buf[b].astype(f32)
                for c in range(NC):
                    xg_buf[b, c] = jnp.broadcast_to(x[:, c * DH:(c + 1) * DH], (G, DH)).astype(bf16)
            y_buf[...] = jnp.zeros(y_buf.shape, f32)

        t = 2 * (i - LAG) - NT
        return lax.cond(t >= 0, lambda: q + q_tile(0, t) + q_tile(0, t + 1), lambda: q)

    q_first = lax.fori_loop(1, NT + LAG, weight_step, zeros)

    def group(grp, carry):
        q, o_prev = (c.astype(bf16) for c in carry)
        prev = jnp.maximum(grp - 1, 0)

        def k_step(t, m):
            wait_kv(t)
            outs = []
            for n in range(P):
                start_ahead(2 * grp, t, n, False)
                outs.append(lax.dot_general(q, tile(t, n), (((1,), (1,)), ((), ())),
                                            preferred_element_type=f32))
            h, c = t >> 2, t & 3
            w = wo_buf[prev, pl.ds(8 * (h & 7), 8), h >> 3, :, pl.ds(pl.multiple_of(c * DH, DH), DH)]
            y = jnp.dot(o_prev, w.reshape(DH, DH), preferred_element_type=f32)
            y_buf[prev >> 1, c] += jnp.where(row == jnp.where(grp > 0, row_of(h), -1), y, 0.0)
            s = own_rows(outs)
            s = jnp.where(even_lanes, s[:P], s[P:]) * (DH ** -0.5)
            s_buf[t] = s
            return jnp.maximum(m, s)

        m = lax.fori_loop(0, NT, k_step, jnp.full((P, 2 * T), -jnp.inf, f32))
        m = jnp.where(even_lanes,
                      jnp.max(jnp.where(even_lanes, m, -jnp.inf), axis=1, keepdims=True),
                      jnp.max(jnp.where(even_lanes, -jnp.inf, m), axis=1, keepdims=True))

        def v_step(t, carry):
            l, acc, q_next = carry
            wait_kv(t)
            p = jnp.exp(s_buf[t] - m)
            p = jnp.concatenate([jnp.where(even_lanes, p, 0.0), jnp.where(even_lanes, 0.0, p)], axis=0)
            p_bf16 = p.astype(bf16)
            outs = []
            for n in range(P):
                start_ahead(2 * grp + 1, t, n, True)
                outs.append(jnp.dot(p_bf16, tile(t, n), preferred_element_type=f32))
            return l + p, acc + own_rows(outs), q_next + q_tile((grp + 1) & (NGRP - 1), t)

        l, acc, q_next = lax.fori_loop(0, NT, v_step, (zeros, zeros, zeros))
        return q_next, acc / jnp.sum(l, axis=1, keepdims=True)

    _, o_last = lax.fori_loop(0, NGRP, group, (q_first, zeros))

    o_buf[...] = o_last
    y_a, y_b = (
        jnp.concatenate([jnp.sum(y_buf[b, c], axis=0, keepdims=True) for c in range(NC)], axis=1)
        for b in range(2))

    def last_step(t, y):
        o = [o_buf[pl.ds(row_of(t + 8 * e), 1), :].astype(bf16) for e in range(2)]
        rows = wo_buf.at[NGRP - 1, pl.ds(8 * t, 8)]
        copy(rows, rows, t).wait()
        for e in range(2):
            w = wo_buf[NGRP - 1, pl.ds(8 * t, 8), e].reshape(DH, D)
            y = y + jnp.dot(o[e], w, preferred_element_type=f32)
        return y

    y_b = lax.fori_loop(0, P, last_step, y_b)
    out_ref[0] = jnp.concatenate([y_a, y_b], axis=1).astype(out_ref.dtype)


@jax.jit
def pallas_concat_heads__mha_block_cached__gqa_block_cached__decode_kernel(
    A_x: jax.Array,
    A_k_cache: jax.Array,
    A_v_cache: jax.Array,
    A_wq: jax.Array,
    A_wo: jax.Array,
    B_x: jax.Array,
    B_k_cache: jax.Array,
    B_v_cache: jax.Array,
    B_wq: jax.Array,
    B_wo: jax.Array,
):
    kv = lambda a: a.reshape(H // 2, 2, NT, T, DH)
    wq = lambda a: a.reshape(2, 2, DH, H * DH)
    wo = lambda a: a.reshape(2, 2, NT, 16, D)
    return pl.pallas_call(
        _kernel,
        out_shape=jax.ShapeDtypeStruct((1, 1, 2 * D), A_x.dtype),
        in_specs=[pl.BlockSpec(memory_space=pltpu.HBM)] * 10,
        out_specs=pl.BlockSpec(memory_space=pltpu.VMEM),
        scratch_shapes=[
            pltpu.VMEM((NSLOT, P, 2, T, DH), jnp.bfloat16),
            pltpu.VMEM((NGRP, 2, 2, DH, G * DH), jnp.bfloat16),
            pltpu.VMEM((NGRP, NT, 2, 16, D), jnp.bfloat16),
            pltpu.VMEM((2, 1, D), jnp.bfloat16),
            pltpu.VMEM((2, NC, G, DH), jnp.bfloat16),
            pltpu.VMEM((NT, P, 2 * T), jnp.float32),
            pltpu.VMEM((2, NC, G, DH), jnp.float32),
            pltpu.VMEM((G, DH), jnp.float32),
            pltpu.SemaphoreType.DMA((NSLOT,)),
            pltpu.SemaphoreType.DMA(()),
        ],
        compiler_params=pltpu.CompilerParams(
            vmem_limit_bytes=32 * 1024 * 1024,
            disable_bounds_checks=True,
            disable_semaphore_checks=True,
        ),
    )(A_x, kv(A_k_cache), kv(A_v_cache), wq(A_wq), wo(A_wo),
      B_x, kv(B_k_cache), kv(B_v_cache), wq(B_wq), wo(B_wo))
```
